```python
import os as _os
_os.environ.setdefault('JAX_PLATFORMS', 'cpu')
import jax
import jax.numpy as jnp

def _softmax(x, axis=-1):
    return jax.nn.softmax(x, axis=axis)

def _gelu(x):
    return jax.nn.gelu(x, approximate=True)

def _silu(x):
    return jax.nn.silu(x)

def _sigmoid(x):
    return jax.nn.sigmoid(x)

def _layernorm(x, axis=-1, eps=1e-05):
    m = jnp.mean(x, axis=axis, keepdims=True)
    v = jnp.var(x, axis=axis, keepdims=True)
    return (x - m) / jnp.sqrt(v + eps)

def _scatter_add(tgt, idx, src, axis=0):
    return tgt.at[idx].add(src)

def _segment_sum(src, seg, n):
    return jax.ops.segment_sum(src, seg, n)

class _Rng:

    def __init__(self, key):
        self._k = key

    def _next(self):
        self._k, sub = jax.random.split(self._k)
        return sub

    def normal(self, shape):
        return jax.random.normal(self._next(), shape, dtype=jnp.bfloat16)

    def randint(self, lo, hi, shape):
        return jax.random.randint(self._next(), shape, lo, hi, dtype=jnp.int32)

    def uniform(self, shape, lo=0.0, hi=1.0):
        return jax.random.uniform(self._next(), shape, jnp.bfloat16, lo, hi)

    def permutation(self, n):
        return jax.random.permutation(self._next(), n)
kernel_name = 'standalone__conformer_conv_module__speech'

def setup_inputs():
    _rng = _Rng(jax.random.key(int.from_bytes(__import__("os").urandom(4), "little")))
    _w = lambda a: (lambda t: t.astype(jnp.bfloat16) if jnp.issubdtype(t.dtype, jnp.floating) else t)(jnp.asarray(a))
    B, T, D, K = (2, 16000, 256, 5)
    return {'x': _w((lambda *s: _rng.normal(s) * 0.2)(B, T, D)), 'w_pw1': _w((lambda *s: _rng.normal(s) * 0.2)(D, 2 * D)), 'dw': _w((lambda *s: _rng.normal(s) * 0.05)(K, D)), 'w_pw2': _w((lambda *s: _rng.normal(s) * 0.05)(D, D))}

def reference(x, w_pw1, dw, w_pw2):
    B, T, D = x.shape
    K = dw.shape[0]
    h = x @ w_pw1
    a, b = (h[..., :D].copy(), h[..., D:].copy())
    h = a * _sigmoid(b)
    pad = K // 2
    hp = jnp.pad(h, ((0, 0), (pad, pad), (0, 0)))
    out = jnp.zeros_like(h)
    for i in range(K):
        out = out + hp[:, i:i + T, :] * dw[i][None, None, :]
    return _silu(out) @ w_pw2
```

```python
import functools

import jax
import jax.numpy as jnp
from jax import lax
import jax.experimental.pallas as pl
import jax.experimental.pallas.tpu as pltpu

LANES = 128
GAP = 16
HEAD = 24


def _plan(rows_per_batch, batch):
    best = None
    for unit in range(16, 257, 16):
        if rows_per_batch % unit == 0:
            best = unit
    unit = best
    per_batch = rows_per_batch // unit
    total = batch * per_batch
    target_loop = max(1, 12480 // unit)
    full = [max(1, round(s * 208 / unit)) for s in (1, 3, 8, 22)]
    for n_ramp in range(len(full), 0, -1):
        ramp = full[:n_ramp]
        if sum(ramp) > per_batch:
            continue
        for extra in range(per_batch - sum(ramp) + 1):
            rest = total - sum(ramp) - extra
            if rest == 0:
                return unit, tuple(ramp[:-1] + [ramp[-1] + extra]), 0
            n_iter = -(-rest // target_loop)
            if rest % n_iter == 0:
                return unit, tuple(ramp[:-1] + [ramp[-1] + extra]), rest // n_iter
    return unit, (per_batch,), per_batch


def _kernel(x_hbm, w1_hbm, dw_hbm, w2_hbm, o_hbm,
            xv, ov, h0, h1, w1s, w1v, dwv, w2v, xsem, osem, wsem,
            *, B, T, D, K, U, ramp, R, piece):
    pad = K // 2
    TV = T + GAP
    NU = TV // U
    G = B * NU
    A = sum(ramp)
    N = (G - A) // R if R else 0
    halves = range(D // LANES)
    hs = (h0, h1)
    base = HEAD - GAP - pad
    edges = [sum(ramp[:k]) for k in range(len(ramp) + 1)] + [A + (i + 1) * R for i in range(N)]
    n_chunks = len(edges) - 1

    def aligned(v):
        return v if isinstance(v, int) else pl.multiple_of(v, 16)

    def x_copies(k):
        copies = []
        for b in range(B):
            u0, u1 = max(edges[k] - b * NU, 0), min(edges[k + 1] - b * NU, NU)
            if u1 > u0:
                r0, r1 = u0 * U, min(u1 * U, T)
                copies.append(pltpu.make_async_copy(
                    x_hbm.at[pl.ds(b * T + r0, r1 - r0), :],
                    xv.at[pl.ds(b * TV + r0, r1 - r0), :], xsem.at[k, b]))
        return copies

    def out_copy(src_row, dst_row, n):
        return pltpu.make_async_copy(ov.at[pl.ds(aligned(src_row), n), :],
                                     o_hbm.at[pl.ds(aligned(dst_row), n), :], osem.at[0])

    def send_static(u0, u1):
        for b in range(B):
            a0, a1 = max(u0 - b * NU, 0), min(u1 - b * NU, NU)
            if a1 > a0:
                r0 = max(a0 * U, GAP)
                out_copy(b * TV + r0, b * T + r0 - GAP, a1 * U - r0).start()

    def send_unit(unit):
        b = jnp.int32(0)
        for k in range(1, B):
            b = b + (unit >= k * NU).astype(jnp.int32)
        inner = out_copy(unit * U, unit * U - (b + 1) * GAP, U)
        first = out_copy(unit * U + GAP, b * T, U - GAP)

        @pl.when(unit != b * NU)
        def _():
            inner.start()

        @pl.when(unit == b * NU)
        def _():
            first.start()

    requested = [0]

    def request(upto):
        while requested[0] < min(upto, n_chunks):
            for c in x_copies(requested[0]):
                c.start()
            requested[0] += 1

    w_copies = [pltpu.make_async_copy(w1_hbm, w1v, wsem.at[0]),
                pltpu.make_async_copy(dw_hbm, dwv, wsem.at[1]),
                pltpu.make_async_copy(w2_hbm, w2v, wsem.at[2])]
    w_copies[0].start()
    request(1)
    w_copies[1].start()
    w_copies[2].start()
    for b in range(B):
        xv[pl.ds(b * TV + T, GAP), :] = jnp.zeros((GAP, D), xv.dtype)
    for j in halves:
        hs[j][pl.ds(0, HEAD), :] = jnp.zeros((HEAD, LANES), jnp.float32)
    w_copies[0].wait()
    request(2)
    w1s[...] = (w1v[...].astype(jnp.float32) * 0.5).astype(w1s.dtype)
    w_copies[1].wait()
    w_copies[2].wait()
    dw_half = dwv[...].astype(jnp.float32) * 0.5
    taps = [[dw_half[i:i + 1, j * LANES:(j + 1) * LANES] for j in halves] for i in range(K)]

    def glu(x_row, h_row, n):
        xb = xv[pl.ds(aligned(x_row), n), :]
        for j in halves:
            a = jnp.dot(xb, w1s[:, j * LANES:(j + 1) * LANES], preferred_element_type=jnp.float32)
            g = jnp.dot(xb, w1s[:, D + j * LANES:D + (j + 1) * LANES], preferred_element_type=jnp.float32)
            hs[j][pl.ds(HEAD + h_row, n), :] = a + a * jnp.tanh(g)

    def conv_silu_proj(o_row, h_row, n, unit_done):
        ys = []
        for j in halves:
            acc = hs[j][pl.ds(base + h_row, n), :] * taps[0][j]
            for i in range(1, K):
                acc = acc + hs[j][pl.ds(base + h_row + i, n), :] * taps[i][j]
            ys.append((acc + acc * jnp.tanh(acc)).astype(w2v.dtype))
        o = jnp.dot(jnp.concatenate(ys, axis=1), w2v[...], preferred_element_type=jnp.float32)
        o = o.astype(ov.dtype)
        for q in range(0, n, U):
            ov[pl.ds(aligned(o_row + q), U), :] = o[q:q + U]
            if unit_done is not None:
                unit_done((h_row + q) // U)

    def process(row0, lo, hi, unit_done=None):
        for r in range(lo, hi, piece):
            n = min(piece, hi - r)
            glu(row0 + r, r, n)
            conv_silu_proj(row0 + r, r, n, unit_done)

    for k in range(len(ramp)):
        for c in x_copies(k):
            c.wait()
        request(k + 3 if k + 1 < len(ramp) else n_chunks)
        process(0, edges[k] * U, edges[k + 1] * U)
    send_static(0, A)

    if N:
        if A != R:
            for j in halves:
                hs[j][pl.ds(R * U, HEAD), :] = hs[j][pl.ds(A * U, HEAD), :]
        waits = [x_copies(len(ramp) + i) for i in range(N)]

        def body(i, carry):
            for step in range(N):
                @pl.when(i == step)
                def _():
                    for c in waits[step]:
                        c.wait()
            for j in halves:
                hs[j][pl.ds(0, HEAD), :] = hs[j][pl.ds(R * U, HEAD), :]
            unit0 = A + i * R
            process(unit0 * U, 0, R * U, lambda q: send_unit(unit0 + q))
            return carry

        lax.fori_loop(0, N, body, 0)

    pltpu.make_async_copy(o_hbm, o_hbm, osem.at[0]).wait()


@jax.jit
def pallas_standalone__conformer_conv_module__speech_kernel(
    x: jax.Array,
    w_pw1: jax.Array,
    dw: jax.Array,
    w_pw2: jax.Array,
):
    B, T, D = x.shape
    K = dw.shape[0]
    assert D == 2 * LANES and T % 16 == 0 and GAP + K // 2 <= HEAD
    U, ramp, R = _plan(T + GAP, B)
    rows = B * (T + GAP)
    n_chunks = len(ramp) + ((rows // U - sum(ramp)) // R if R else 0)
    h_rows = max(sum(ramp), R) * U + HEAD
    hbm = pl.BlockSpec(memory_space=pl.ANY)

    out = pl.pallas_call(
        functools.partial(_kernel, B=B, T=T, D=D, K=K, U=U, ramp=ramp, R=R, piece=5 * U),
        out_shape=jax.ShapeDtypeStruct((B * T, D), x.dtype),
        in_specs=[hbm, hbm, hbm, hbm],
        out_specs=hbm,
        scratch_shapes=[
            pltpu.VMEM((rows, D), x.dtype),
            pltpu.VMEM((rows, D), x.dtype),
            pltpu.VMEM((h_rows, LANES), jnp.float32),
            pltpu.VMEM((h_rows, LANES), jnp.float32),
            pltpu.VMEM(w_pw1.shape, w_pw1.dtype),
            pltpu.VMEM(w_pw1.shape, w_pw1.dtype),
            pltpu.VMEM(dw.shape, dw.dtype),
            pltpu.VMEM(w_pw2.shape, w_pw2.dtype),
            pltpu.SemaphoreType.DMA((n_chunks, B)),
            pltpu.SemaphoreType.DMA((1,)),
            pltpu.SemaphoreType.DMA((3,)),
        ],
        compiler_params=pltpu.CompilerParams(
            vmem_limit_bytes=100 * 1024 * 1024,
            disable_bounds_checks=True,
        ),
    )(x.reshape(B * T, D), w_pw1, dw, w_pw2)
    return out.reshape(B, T, D)
```

```python
import functools

import jax
import jax.numpy as jnp
from jax import lax
import jax.experimental.pallas as pl
import jax.experimental.pallas.tpu as pltpu

LANES = 128
GAP = 16
HEAD = 24


def _plan(rows_per_batch, batch):
    unit = max(u for u in range(16, 257, 16) if rows_per_batch % u == 0)
    per_batch = rows_per_batch // unit
    total = batch * per_batch
    target_loop = max(1, 12480 // unit)
    full = [max(1, round(s * 208 / unit)) for s in (1, 3, 8, 22)]
    for n_ramp in range(len(full), 0, -1):
        ramp = full[:n_ramp]
        if sum(ramp) > per_batch:
            continue
        for extra in range(per_batch - sum(ramp) + 1):
            rest = total - sum(ramp) - extra
            if rest == 0:
                return unit, tuple(ramp[:-1] + [ramp[-1] + extra]), 0
            n_iter = -(-rest // target_loop)
            if rest % n_iter == 0:
                return unit, tuple(ramp[:-1] + [ramp[-1] + extra]), rest // n_iter
    return unit, (per_batch,), per_batch


def _kernel(x_hbm, w1_hbm, dw_hbm, w2_hbm, o_hbm,
            xv, ov, h0, h1, w1s, w1v, dwv, w2v, sems,
            *, B, T, D, K, U, ramp, R, piece):
    pad = K // 2
    TV = T + GAP
    NU = TV // U
    G = B * NU
    A = sum(ramp)
    N = (G - A) // R if R else 0
    halves = range(D // LANES)
    hs = (h0, h1)
    base = HEAD - GAP - pad
    edges = [sum(ramp[:k]) for k in range(len(ramp) + 1)] + [A + (i + 1) * R for i in range(N)]
    n_chunks = len(edges) - 1

    def aligned(v):
        return v if isinstance(v, int) else pl.multiple_of(v, 16)

    n_ramp = len(ramp)
    osem = sems.at[2 + N]

    def x_sem(k):
        return sems.at[(k + 1) % 2 if k < n_ramp else 2 + k - n_ramp]

    def x_copies(k):
        copies = []
        for b in range(B):
            u0, u1 = max(edges[k] - b * NU, 0), min(edges[k + 1] - b * NU, NU)
            if u1 > u0:
                r0, r1 = u0 * U, min(u1 * U, T)
                copies.append(pltpu.make_async_copy(
                    x_hbm.at[pl.ds(b * T + r0, r1 - r0), :],
                    xv.at[pl.ds(b * TV + r0, r1 - r0), :], x_sem(k)))
        return copies

    def out_copy(src_row, dst_row, n):
        return pltpu.make_async_copy(ov.at[pl.ds(aligned(src_row), n), :],
                                     o_hbm.at[pl.ds(aligned(dst_row), n), :], osem)

    def send_static(u0, u1):
        for b in range(B):
            a0, a1 = max(u0 - b * NU, 0), min(u1 - b * NU, NU)
            if a1 > a0:
                r0 = max(a0 * U, GAP)
                out_copy(b * TV + r0, b * T + r0 - GAP, a1 * U - r0).start()

    def send_unit(unit):
        b = jnp.int32(0)
        for k in range(1, B):
            b = b + (unit >= k * NU).astype(jnp.int32)
        inner = out_copy(unit * U, unit * U - (b + 1) * GAP, U)
        first = out_copy(unit * U + GAP, b * T, U - GAP)

        @pl.when(unit != b * NU)
        def _():
            inner.start()

        @pl.when(unit == b * NU)
        def _():
            first.start()

    requested = [0]

    def request(upto):
        while requested[0] < min(upto, n_chunks):
            for c in x_copies(requested[0]):
                c.start()
            requested[0] += 1

    w_copies = [pltpu.make_async_copy(w1_hbm, w1v, x_sem(1)),
                pltpu.make_async_copy(dw_hbm, dwv, x_sem(0)),
                pltpu.make_async_copy(w2_hbm, w2v, x_sem(0))]
    w_copies[0].start()
    request(1)
    w_copies[1].start()
    w_copies[2].start()
    for b in range(B):
        xv[pl.ds(b * TV + T, GAP), :] = jnp.zeros((GAP, D), xv.dtype)
    for j in halves:
        hs[j][pl.ds(0, HEAD), :] = jnp.zeros((HEAD, LANES), jnp.float32)
    w_copies[0].wait()
    request(2)
    w1s[...] = (w1v[...].astype(jnp.float32) * 0.5).astype(w1s.dtype)
    for c in w_copies[1:] + x_copies(0):
        c.wait()
    dw_half = dwv[...].astype(jnp.float32) * 0.5
    taps = [[dw_half[i:i + 1, j * LANES:(j + 1) * LANES] for j in halves] for i in range(K)]

    def glu(x_row, h_row, n):
        xb = xv[pl.ds(aligned(x_row), n), :]
        for j in halves:
            a = jnp.dot(xb, w1s[:, j * LANES:(j + 1) * LANES], preferred_element_type=jnp.float32)
            g = jnp.dot(xb, w1s[:, D + j * LANES:D + (j + 1) * LANES], preferred_element_type=jnp.float32)
            hs[j][pl.ds(HEAD + h_row, n), :] = a + a * jnp.tanh(g)

    def conv_silu_proj(o_row, h_row, n, unit_done):
        ys = []
        for j in halves:
            acc = hs[j][pl.ds(base + h_row, n), :] * taps[0][j]
            for i in range(1, K):
                acc = acc + hs[j][pl.ds(base + h_row + i, n), :] * taps[i][j]
            ys.append((acc + acc * jnp.tanh(acc)).astype(w2v.dtype))
        o = jnp.dot(jnp.concatenate(ys, axis=1), w2v[...], preferred_element_type=jnp.float32)
        o = o.astype(ov.dtype)
        for q in range(0, n, U):
            ov[pl.ds(aligned(o_row + q), U), :] = o[q:q + U]
            if unit_done is not None:
                unit_done((h_row + q) // U)

    def process(row0, lo, hi, unit_done=None):
        for r in range(lo, hi, piece):
            n = min(piece, hi - r)
            glu(row0 + r, r, n)
            conv_silu_proj(row0 + r, r, n, unit_done)

    for k in range(n_ramp):
        if k > 0:
            for c in x_copies(k):
                c.wait()
        request(k + 3 if k + 1 < n_ramp else n_chunks)
        process(0, edges[k] * U, edges[k + 1] * U)
    send_static(0, A)

    if N:
        if A != R:
            for j in halves:
                hs[j][pl.ds(R * U, HEAD), :] = hs[j][pl.ds(A * U, HEAD), :]
        waits = [x_copies(n_ramp + i) for i in range(N)]

        def body(i, carry):
            for step in range(N):
                @pl.when(i == step)
                def _():
                    for c in waits[step]:
                        c.wait()
            for j in halves:
                hs[j][pl.ds(0, HEAD), :] = hs[j][pl.ds(R * U, HEAD), :]
            unit0 = A + i * R
            process(unit0 * U, 0, R * U, lambda q: send_unit(unit0 + q))
            return carry

        lax.fori_loop(0, N, body, 0)

    pltpu.make_async_copy(o_hbm, o_hbm, osem).wait()


@jax.jit
def pallas_standalone__conformer_conv_module__speech_kernel(
    x: jax.Array,
    w_pw1: jax.Array,
    dw: jax.Array,
    w_pw2: jax.Array,
):
    B, T, D = x.shape
    K = dw.shape[0]
    assert D == 2 * LANES and T % 16 == 0 and GAP + K // 2 <= HEAD
    U, ramp, R = _plan(T + GAP, B)
    rows = B * (T + GAP)
    n_loop = (rows // U - sum(ramp)) // R if R else 0
    h_rows = max(sum(ramp), R) * U + HEAD
    hbm = pl.BlockSpec(memory_space=pl.ANY)

    out = pl.pallas_call(
        functools.partial(_kernel, B=B, T=T, D=D, K=K, U=U, ramp=ramp, R=R, piece=5 * U),
        out_shape=jax.ShapeDtypeStruct((B * T, D), x.dtype),
        in_specs=[hbm, hbm, hbm, hbm],
        out_specs=hbm,
        scratch_shapes=[
            pltpu.VMEM((rows, D), x.dtype),
            pltpu.VMEM((rows, D), x.dtype),
            pltpu.VMEM((h_rows, LANES), jnp.float32),
            pltpu.VMEM((h_rows, LANES), jnp.float32),
            pltpu.VMEM(w_pw1.shape, w_pw1.dtype),
            pltpu.VMEM(w_pw1.shape, w_pw1.dtype),
            pltpu.VMEM(dw.shape, dw.dtype),
            pltpu.VMEM(w_pw2.shape, w_pw2.dtype),
            pltpu.SemaphoreType.DMA((n_loop + 3,)),
        ],
        compiler_params=pltpu.CompilerParams(vmem_limit_bytes=100 * 1024 * 1024),
    )(x.reshape(B * T, D), w_pw1, dw, w_pw2)
    return out.reshape(B, T, D)
```
